```python
import os as _os
_os.environ.setdefault("JAX_PLATFORMS", "cpu")
import jax
import jax.numpy as jnp

def _softmax(x, axis=-1):
    return jax.nn.softmax(x, axis=axis)
def _gelu(x):
    return jax.nn.gelu(x, approximate=True)
def _silu(x):
    return jax.nn.silu(x)
def _sigmoid(x):
    return jax.nn.sigmoid(x)
def _layernorm(x, axis=-1, eps=1e-5):
    m = jnp.mean(x, axis=axis, keepdims=True)
    v = jnp.var(x, axis=axis, keepdims=True)
    return (x - m) / jnp.sqrt(v + eps)
def _scatter_add(tgt, idx, src, axis=0):
    return tgt.at[idx].add(src)
def _segment_sum(src, seg, n):
    return jax.ops.segment_sum(src, seg, n)
class _Rng:
    def __init__(self, key):
        self._k = key
    def _next(self):
        self._k, sub = jax.random.split(self._k)
        return sub
    def normal(self, shape):
        return jax.random.normal(self._next(), shape, dtype=jnp.bfloat16)
    def randint(self, lo, hi, shape):
        return jax.random.randint(self._next(), shape, lo, hi, dtype=jnp.int32)
    def uniform(self, shape, lo=0.0, hi=1.0):
        return jax.random.uniform(self._next(), shape, jnp.bfloat16, lo, hi)
    def permutation(self, n):
        return jax.random.permutation(self._next(), n)


kernel_name = 'interleave_layers__mha_block__mixer_s_mlp__prompt'

def setup_inputs():
    _rng = _Rng(jax.random.key(int.from_bytes(__import__("os").urandom(4), "little")))
    _w = (lambda a: (lambda t: t.astype(jnp.bfloat16) if jnp.issubdtype(t.dtype, jnp.floating) else t)(jnp.asarray(a)))
    def _A_setup():
        B, S, D, H = 1, 2048, 448, 16
        return {
            "x": _w((lambda *s: _rng.normal(s) * 0.05)(B, S, D)),
            "wqkv": _w((lambda *s: _rng.normal(s) * 0.05)(D, 3 * D)),
            "wo": _w((lambda *s: _rng.normal(s) * 0.05)(D, D)),
        }
    _A_in = _A_setup()

    def _B_setup():
        B, S, D, F = 1, 2048, 448, 1792
        return {
            "x":  _w((lambda *s: _rng.normal(s) * 0.05)(B, S, D)),
            "w1": _w((lambda *s: _rng.normal(s) * 0.8)(D, D) * (D ** -0.5)),
            "w2": _w((lambda *s: _rng.normal(s) * 0.8)(D, D) * (D ** -0.5)),
            "w3": _w((lambda *s: _rng.normal(s) * 0.8)(D, F) * (D ** -0.5)),
            "w4": _w((lambda *s: _rng.normal(s) * 0.8)(F, D) * (F ** -0.5)),
        }
    _B_in = _B_setup()

    return {
        "A_x": _A_in["x"],
        "A_wqkv": _A_in["wqkv"],
        "A_wo": _A_in["wo"],
        "B_x": _B_in["x"],
        "B_w1": _B_in["w1"],
        "B_w2": _B_in["w2"],
        "B_w3": _B_in["w3"],
        "B_w4": _B_in["w4"],
    }

def reference(A_x, A_wqkv, A_wo, B_x, B_w1, B_w2, B_w3, B_w4):
    def _A_ref(x, wqkv, wo):
        B, S, D = x.shape
        H = 16
        Dh = D // H
        qkv = (lambda x, *d: x.transpose(*d))((x @ wqkv).reshape(B, S, 3, H, Dh), 2, 0, 3, 1, 4)
        q, k, v = qkv[0], qkv[1], qkv[2]
        scores = jnp.einsum("bhqd,bhkd->bhqk", q, k) * (Dh ** -0.5)
        p = _softmax(scores, axis=-1)
        o = jnp.einsum("bhqk,bhkd->bhqd", p, v)
        return (lambda x, *d: x.transpose(*d))(o, 0, 2, 1, 3).reshape(B, S, D) @ wo

    def _B_ref(x, w1, w2, w3, w4):
        B, S, D = x.shape
        h = _gelu(_layernorm(x, axis=-1) @ w1)
        c = D // 4
        g0 = jnp.pad(h[:, :, 0*c:1*c], ((0, 0), (1, 0), (0, 0)))[:, :S, :]
        g1 = jnp.pad(h[:, :, 1*c:2*c], ((0, 0), (0, 1), (0, 0)))[:, 1:, :]
        g2 = jnp.pad(h[:, :, 2*c:3*c], ((0, 0), (2, 0), (0, 0)))[:, :S, :]
        g3 = jnp.pad(h[:, :, 3*c:   ], ((0, 0), (0, 2), (0, 0)))[:, 2:, :]
        hs = jnp.concatenate([g0, g1, g2, g3], axis=-1) @ w2
        x1 = x + hs
        h2 = _gelu(_layernorm(x1, axis=-1) @ w3) @ w4
        return x1 + h2

    x = A_x
    x = x + _A_ref(_layernorm(x, axis=-1), A_wqkv, A_wo)
    x = x + _B_ref(_layernorm(x, axis=-1), B_w1, B_w2, B_w3, B_w4)
    x = x + _A_ref(_layernorm(x, axis=-1), A_wqkv, A_wo)
    x = x + _B_ref(_layernorm(x, axis=-1), B_w1, B_w2, B_w3, B_w4)
    return x
```

```python
import math

import jax
import jax.numpy as jnp
from jax import lax
from jax.experimental import pallas as pl
from jax.experimental.pallas import tpu as pltpu

f32 = jnp.float32
bf16 = jnp.bfloat16

S, D, H, F = 2048, 448, 16, 1792
DH = D // H
WIN = 32
EPS = 1e-5
QSCALE = DH ** -0.5 * math.log2(math.e)
PADL = 128

DEFAULT = dict(T=512, C=128, U=1, LAG=1, K32=0, P4L=0, P1L=0, P3L=0, FLAG=0)


def _dot(a, b):
    return jnp.dot(a, b, preferred_element_type=f32)


def _ln(x):
    mean = jnp.sum(x, axis=0, keepdims=True) * (1.0 / D)
    xc = x - mean
    var = jnp.sum(xc * xc, axis=0, keepdims=True) * (1.0 / D)
    return xc * lax.rsqrt(var + EPS)


def _gelu(x):
    c = math.sqrt(2.0 / math.pi)
    u = x * (x * x * (c * 0.044715) + c)
    hx = 0.5 * x
    return hx * jnp.tanh(u) + hx


def _win_start(h):
    return (DH * h) // 8 * 8


def _own_rows(h, width):
    r = lax.broadcasted_iota(jnp.int32, (WIN, width), 0)
    off = DH * h - _win_start(h)
    return (r >= off) & (r < off + DH)


def make(**cfg):
    P = dict(DEFAULT)
    P.update(cfg)
    T, C, U, LAG = P['T'], P['C'], P['U'], P['LAG']
    NT = S // T
    NC = S // C

    def kern(x_hbm, wqkv_hbm, wo_hbm, w1_hbm, w2_hbm, w3_hbm, w4_hbm, out_hbm,
             xin, wqkv_in, wo_in, w1_in, w2_in, w3_in, w4t,
             wqkvt, wot, w1t, w2t, w3t,
             x_ref, y_ref, q_ref, k_ref, v_ref, o_ref, s_ref, h_ref, outb,
             in_sem, out_sem):

        def in_copy(src, dst, i):
            return pltpu.make_async_copy(src, dst, in_sem.at[i])

        x_cp = [in_copy(x_hbm.at[:, pl.ds(j * T, T)], xin.at[:, pl.ds(j * T, T)], j) for j in range(NT)]
        wqkv_cp = in_copy(wqkv_hbm, wqkv_in, NT)
        wo_cp = in_copy(wo_hbm, wo_in, NT + 1)
        w1_cp = in_copy(w1_hbm, w1_in, NT + 2)
        w2_cp = in_copy(w2_hbm, w2_in, NT + 3)
        w3_cp = in_copy(w3_hbm, w3_in, NT + 4)
        w4_cp = in_copy(w4_hbm, w4t, NT + 5)
        wqkv_cp.start()
        for cp in x_cp:
            cp.start()
        for cp in (wo_cp, w1_cp, w2_cp, w3_cp, w4_cp):
            cp.start()

        h_ref[:, 0:PADL] = jnp.zeros((D, PADL), bf16)
        h_ref[:, PADL + S:] = jnp.zeros((D, PADL), bf16)
        if not P['K32']:
            q_ref[...] = jnp.zeros(q_ref.shape, bf16)

        wqkv_cp.wait()
        wqkvt[...] = wqkv_in[...].T
        for j in range(NT):
            x_cp[j].wait()
            x_ref[:, j * T:(j + 1) * T] = xin[:, j * T:(j + 1) * T].astype(f32)

        def cols(j):
            if isinstance(j, int):
                return slice(j * T, (j + 1) * T)
            return pl.ds(pl.multiple_of(j * T, T), T)

        def p1_ln(j):
            return _ln(x_ref[:, cols(j)]).astype(bf16)

        def p1_q(j, xn):
            q = _dot(wqkvt[0:D, :], xn) * QSCALE
            for h in range(H):
                r0 = _win_start(h)
                w = jnp.where(_own_rows(h, T), q[r0:r0 + WIN], 0.0)
                if P['K32']:
                    q_ref[h, :, cols(j)] = w.astype(bf16)
                else:
                    g0 = r0 - 112 * (h // 4)
                    a0 = g0 // 16 * 16
                    a1 = (g0 + WIN + 15) // 16 * 16
                    parts = []
                    if g0 > a0:
                        parts.append(jnp.zeros((g0 - a0, T), f32))
                    parts.append(w)
                    if a1 > g0 + WIN:
                        parts.append(jnp.zeros((a1 - g0 - WIN, T), f32))
                    q_ref[h, a0:a1, cols(j)] = jnp.concatenate(parts, axis=0).astype(bf16)

        def p1_k(j, xn):
            k = _dot(wqkvt[D:2 * D, :], xn)
            if P['K32']:
                for h in range(H):
                    r0 = _win_start(h)
                    k_ref[h, cols(j), :] = k[r0:r0 + WIN].astype(bf16).T
            else:
                kb = k.astype(bf16)
                for g in range(4):
                    kg = jnp.concatenate([kb[112 * g:112 * g + 112], jnp.zeros((16, T), bf16)], axis=0)
                    k_ref[g, cols(j), :] = kg.T

        def p1_v(j, xn):
            v = _dot(wqkvt[2 * D:3 * D, :], xn)
            for h in range(H):
                r0 = _win_start(h)
                v_ref[h, :, cols(j)] = jnp.where(_own_rows(h, T), v[r0:r0 + WIN], 1.0).astype(bf16)

        def phase1():
            if P['P1L']:
                def body(j, c):
                    xn = p1_ln(j)
                    p1_k(j, xn)
                    p1_v(j, xn)
                    p1_q(j, xn)
                    return c
                lax.fori_loop(0, NT, body, 0)
            else:
                xn = p1_ln(0)
                for j in range(NT):
                    p1_k(j, xn)
                    nxt = p1_ln(j + 1) if j + 1 < NT else None
                    p1_v(j, xn)
                    p1_q(j, xn)
                    xn = nxt

        def scores(h, j, c, buf, m):
            kk = k_ref[h, c * C:(c + 1) * C, :] if P['K32'] else k_ref[h // 4, c * C:(c + 1) * C, :]
            s = _dot(kk, q_ref[h, :, cols(j)])
            s_ref[buf, c * C:(c + 1) * C, :] = s
            cm = jnp.max(s.reshape(C // 8, 8, T), axis=0)
            return cm if m is None else jnp.maximum(m, cm)

        def pv(h, c, buf, m, acc):
            p = jnp.exp2(s_ref[buf, c * C:(c + 1) * C, :] - m).astype(bf16)
            a = _dot(v_ref[h, :, c * C:(c + 1) * C], p)
            return a if acc is None else acc + a

        def finish(h, j, acc):
            if isinstance(h, int):
                l = acc[WIN - 1:WIN] if h % 2 == 0 else acc[0:1]
            else:
                l = jnp.where(h % 2 == 0, acc[WIN - 1:WIN], acc[0:1])
            o = (acc * (1.0 / l)).astype(bf16)
            if isinstance(h, int):
                o_ref[h * WIN:(h + 1) * WIN, cols(j)] = o
            else:
                o_ref[pl.ds(pl.multiple_of(h * WIN, WIN), WIN), cols(j)] = o

        def phase2():
            m8 = None
            for c in range(NC):
                m8 = scores(0, 0, c, 0, m8)
            head = None
            for c in range(LAG):
                head = scores(0, 1, c, 1, head)

            def unit(h, j, m8, head):
                cur, nxt = j % 2, 1 - j % 2
                hn, jn = (h, j + 1) if j + 1 < NT else (jnp.minimum(h + 1, H - 1), 0)
                hnn, jnn = (h, j + 2) if j + 2 < NT else (jnp.minimum(h + 1, H - 1), j + 2 - NT)
                m = jnp.max(m8, axis=0, keepdims=True)
                acc = None
                mn, head2 = head, None
                for c in range(NC):
                    if c + LAG < NC:
                        mn = scores(hn, jn, c + LAG, nxt, mn)
                    acc = pv(h, c, cur, m, acc)
                    if c + LAG >= NC:
                        head2 = scores(hnn, jnn, c + LAG - NC, cur, head2)
                finish(h, j, acc)
                return mn, head2

            def body(i, carry):
                m8, head = carry
                for u in range(U):
                    for j in range(NT):
                        m8, head = unit(i * U + u, j, m8, head)
                return m8, head

            lax.fori_loop(0, H // U, body, (m8, head))

        def p3_wo(j):
            x = x_ref[:, cols(j)] + _dot(wot[...], o_ref[:, cols(j)])
            x_ref[:, cols(j)] = x
            y = _ln(x)
            y_ref[:, cols(j)] = y
            return _ln(y).astype(bf16)

        def p3_w1(j, z):
            hh = _gelu(_dot(w1t[...], z)).astype(bf16)
            if isinstance(j, int):
                h_ref[:, PADL + j * T:PADL + (j + 1) * T] = hh
            else:
                h_ref[:, pl.ds(pl.multiple_of(PADL + j * T, PADL), T)] = hh

        def phase3():
            z = p3_wo(0)
            for j in range(NT):
                nxt = p3_wo(j + 1) if j + 1 < NT else None
                p3_w1(j, z)
                z = nxt

        def p4_w2(j):
            parts = []
            for c, sh in enumerate((1, -1, 2, -2)):
                if isinstance(j, int):
                    win = h_ref[112 * c:112 * (c + 1), j * T:j * T + T + 2 * PADL]
                else:
                    win = h_ref[112 * c:112 * (c + 1), pl.ds(pl.multiple_of(j * T, PADL), T + 2 * PADL)]
                parts.append(win[:, PADL - sh:PADL - sh + T])
            g = jnp.concatenate(parts, axis=0)
            x1 = y_ref[:, cols(j)] + _dot(w2t[...], g)
            x_ref[:, cols(j)] = x_ref[:, cols(j)] + x1
            return _ln(x1).astype(bf16)

        def p4_w3(j, u):
            return _gelu(_dot(w3t[...], u)).astype(bf16)

        def p4_w4(j, hid):
            x = x_ref[:, cols(j)] + _dot(w4t[...], hid)
            x_ref[:, cols(j)] = x
            outb[:, cols(j)] = x.astype(bf16)

        def phase4():
            if P['P4L']:
                n = P['P4L']

                def body(i, c):
                    us = [p4_w2(i * n + a) for a in range(n)]
                    hids = [p4_w3(i * n + a, us[a]) for a in range(n)]
                    for a in range(n):
                        p4_w4(i * n + a, hids[a])
                    return c
                lax.fori_loop(0, NT // n, body, 0)
            else:
                u = p4_w2(0)
                hid = None
                for j in range(NT):
                    un = p4_w2(j + 1) if j + 1 < NT else None
                    hn = p4_w3(j, u)
                    if hid is not None:
                        p4_w4(j - 1, hid)
                    hid, u = hn, un
                p4_w4(NT - 1, hid)

        def prep_weights():
            wo_cp.wait()
            wo = wo_in[...].astype(f32)
            wins = []
            for h in range(H):
                r0 = _win_start(h)
                wins.append(jnp.where(_own_rows(h, D), wo[r0:r0 + WIN], 0.0))
            wot[...] = jnp.concatenate(wins, axis=0).astype(bf16).T
            w1_cp.wait()
            w1t[...] = w1_in[...].T
            w2_cp.wait()
            w2t[...] = w2_in[...].T
            w3_cp.wait()
            w3t[...] = w3_in[...].T
            w4_cp.wait()

        def layer(l, c):
            phase1()

            @pl.when(l == 0)
            def _():
                prep_weights()

            phase2()
            phase3()
            phase4()
            return c

        lax.fori_loop(0, 2, layer, 0)

        cps = [pltpu.make_async_copy(outb.at[:, pl.ds(j * T, T)], out_hbm.at[:, pl.ds(j * T, T)], out_sem.at[j])
               for j in range(NT)]
        for cp in cps:
            cp.start()
        for cp in cps:
            cp.wait()

    flags = {}
    if P['FLAG'] == 1:
        flags = {"XLA_TPU_FORCE_LP_LLO_SCHEDULER": True}

    kshape = (H, S, WIN) if P['K32'] else (4, S, 128)
    qshape = (H, WIN, S) if P['K32'] else (H, 128, S)

    def fn(A_x, A_wqkv, A_wo, B_x, B_w1, B_w2, B_w3, B_w4):
        del B_x
        any_spec = pl.BlockSpec(memory_space=pl.ANY)
        out = pl.pallas_call(
            kern,
            out_shape=jax.ShapeDtypeStruct((D, S), bf16),
            in_specs=[any_spec] * 7,
            out_specs=any_spec,
            scratch_shapes=[
                pltpu.VMEM((D, S), bf16),
                pltpu.VMEM((D, 3 * D), bf16),
                pltpu.VMEM((D, D), bf16),
                pltpu.VMEM((D, D), bf16),
                pltpu.VMEM((D, D), bf16),
                pltpu.VMEM((D, F), bf16),
                pltpu.VMEM((D, F), bf16),
                pltpu.VMEM((3 * D, D), bf16),
                pltpu.VMEM((D, H * WIN), bf16),
                pltpu.VMEM((D, D), bf16),
                pltpu.VMEM((D, D), bf16),
                pltpu.VMEM((F, D), bf16),
                pltpu.VMEM((D, S), f32),
                pltpu.VMEM((D, S), f32),
                pltpu.VMEM(qshape, bf16),
                pltpu.VMEM(kshape, bf16),
                pltpu.VMEM((H, WIN, S), bf16),
                pltpu.VMEM((H * WIN, S), bf16),
                pltpu.VMEM((2, S, T), f32),
                pltpu.VMEM((D, S + 2 * PADL), bf16),
                pltpu.VMEM((D, S), bf16),
                pltpu.SemaphoreType.DMA((NT + 6,)),
                pltpu.SemaphoreType.DMA((NT,)),
            ],
            compiler_params=pltpu.CompilerParams(vmem_limit_bytes=110 * 2 ** 20, flags=flags),
            name='fused',
        )(A_x[0].T, A_wqkv, A_wo, B_w1, B_w2, B_w3, B_w4.T)
        return out.T[None]

    return jax.jit(fn)


_kernel = make()


@jax.jit
def pallas_interleave_layers__mha_block__mixer_s_mlp__prompt_kernel(A_x, A_wqkv, A_wo, B_x, B_w1, B_w2, B_w3, B_w4):
    return _kernel(A_x, A_wqkv, A_wo, B_x, B_w1, B_w2, B_w3, B_w4)
```

```python
import math

import jax
import jax.numpy as jnp
from jax import lax
import jax.experimental.pallas as pl
import jax.experimental.pallas.tpu as pltpu

f32, bf16, u32 = jnp.float32, jnp.bfloat16, jnp.uint32

S, D, H, F = 2048, 448, 16, 1792
DH = D // H
D2, F2 = D // 2, F // 2
GRP = 4 * DH
WIN = 32
LANE = 128
EPS = 1e-5
QSCALE = DH ** -0.5 * math.log2(math.e)
GELU_C = math.sqrt(2.0 / math.pi)
SHIFTS = (1, -1, 2, -2)

T = 1024
TH = T // 2
W = 512
NW = S // W
C = 128
NC = S // C
HID = 256
FA, FB = 512, 384
DEPTH = (FA, FB, FB, FA, FB, FA, FA)


def _dot(a, b):
    return jnp.dot(a, b, preferred_element_type=f32)


def _pack(v):
    return pltpu.bitcast(v.astype(bf16), u32)


def _pack_mixed(v):
    n, m = v.shape
    v = v.reshape(n // 16, 2, 8, m)
    return pltpu.pack_elementwise([v[:, 0].reshape(n // 2, m), v[:, 1].reshape(n // 2, m)], packed_dtype=bf16)


def _unpack(w):
    return pltpu.bitcast(w, bf16)


def _mixed(w):
    return _unpack(_pack_mixed(w)).astype(f32)


def _unmixed(w):
    n, m = w.shape
    words = _pack(w)
    parts = [pltpu.unpack_elementwise(words, index=i, packed_dtype=bf16, unpacked_dtype=f32).reshape(n // 16, 1, 8, m)
             for i in range(2)]
    return jnp.concatenate(parts, axis=1).reshape(n, m)


def _words(r0, n):
    return slice(r0 // 2, (r0 + n) // 2)


def _gelu(x):
    hx = 0.5 * x
    return hx * jnp.tanh(x * (x * x * (GELU_C * 0.044715) + GELU_C)) + hx


def _win_start(h):
    return (DH * h) // 8 * 8


def _own_rows(h, width):
    r = lax.broadcasted_iota(jnp.int32, (WIN, width), 0)
    off = DH * h - _win_start(h)
    return (r >= off) & (r < off + DH)


def _lhs(a11, a12, a21, a22):
    return a21 + a22, a22, a11 + a12, a11 + a22, a12 - a22, a11, a21 - a11


def _rhs(b11, b12, b21, b22):
    return b11, b21 - b11, b22, b11 + b22, b21 + b22, b12 - b22, b11 + b12


def _block(i, m):
    if i == 0:
        return (m[1] - m[2]) + m[3] + m[4]
    if i == 1:
        return m[5] + m[2]
    if i == 2:
        return m[0] + m[1]
    return (m[3] - m[0]) + m[5] + m[6]


def _put_lhs(a_ref, r0, *blocks):
    for i, v in enumerate(_lhs(*blocks)):
        a_ref[i, _words(r0, v.shape[0]), :] = _pack(v)


def _put_rhs(b_ref, r0, cols, *blocks):
    for i, v in enumerate(_rhs(*blocks)):
        b_ref[i, _words(r0, v.shape[0]), cols] = _pack_mixed(v)


def _matmul(a_ref, b_ref, chunk, now, later=None, paced=()):
    twice = len(a_ref.shape) == 4
    total = 4 * a_ref.shape[2] if twice else 2 * a_ref.shape[1]
    due, todo = {}, []
    for funcs, (begin, end) in paced:
        for k, f in enumerate(funcs):
            due.setdefault(int(total * 7 // 8 * (begin + (end - begin) * k / len(funcs))), []).append(f)
    starts = [0] + list(range(total % chunk or chunk, total + 1, chunk))
    for r0, r1 in zip(starts, starts[1:]):
        rows, m = r1 - r0, []
        for k, f in enumerate(todo):
            due.setdefault((r0 * 7 + rows * 7 * k // len(todo)) // 8, []).append(f)
        for i in range(7):
            if twice:
                p = [_dot(_unpack(a_ref[i, k, :, 0:n]), _unpack(b_ref[i, k, 0:n // 2, :])) for k, n in enumerate(DEPTH)]
                c = [_block(k, p) for k in range(4)]
                m.append(jnp.concatenate([jnp.concatenate(c[0:2], axis=1), jnp.concatenate(c[2:4], axis=1)], axis=0))
            else:
                m.append(_dot(_unpack(a_ref[i, _words(r0, rows), :]), _unpack(b_ref[i])))
            for r in range(0, rows, 8):
                for f in due.get((r0 * 7 + i * rows + r) // 8, ()):
                    f(p[r // 32][r % 32 * 3:r % 32 * 3 + 8, 0:LANE] if twice else m[i][r:r + 8, 0:LANE])
            done = {1: 2, 4: 0, 5: 1, 6: 3}.get(i)
            if done is not None:
                now(r0, done, _block(done, m))
        todo = later(r0, rows) if later is not None else []
    return todo


def _kernel(x_hbm, wqkv_hbm, wo_hbm, w1_hbm, w2_hbm, w3_hbm, w4_hbm, out_hbm,
            io_buf, wqkv_in, wo_in, w1_in, w2_in, w3_in, w4_in,
            a_qkv, a_o, a_1, a_2, a_3, a_4,
            b_d, b_o, b_f0, b_f1, g_ref0, g_ref1, g_ref2, one_ref, stat_ref,
            x_ref, y_ref, q_ref, k_ref, v_ref, o_ref, s_ref0, s_ref1, h_ref,
            in_sem, out_sem):
    b_f, g_ref, s_ref = (b_f0, b_f1), (g_ref0, g_ref1, g_ref2), (s_ref0, s_ref1)

    x_cp = [pltpu.make_async_copy(x_hbm.at[:, pl.ds(j * T, T)], io_buf.at[:, pl.ds(j * T, T)], in_sem.at[6 + j])
            for j in range(2)]
    w_cp = [pltpu.make_async_copy(src, dst, in_sem.at[i]) for i, (src, dst) in enumerate((
        (wqkv_hbm, wqkv_in), (wo_hbm, wo_in), (w1_hbm, w1_in), (w2_hbm, w2_in), (w3_hbm, w3_in), (w4_hbm, w4_in)))]

    def out_copy(j, i):
        at = (pl.ds(i // 2 * D2, D2), pl.ds(j * T + i % 2 * TH, TH))
        return pltpu.make_async_copy(io_buf.at[at], out_hbm.at[at], out_sem.at[4 * j + i])

    def fence():
        def body(i, carry):
            one_ref[i] = jnp.ones((8, LANE), f32)
            return carry
        lax.fori_loop(0, 2, body, 0)

    def after(v, gate):
        if gate is None:
            return v
        n, m = v.shape
        full = m // LANE * LANE
        parts = [jnp.where(one_ref[0] > 0.0, v[:, t:t + LANE].reshape(n // 8, 8, LANE), gate).reshape(n, LANE)
                 for t in range(0, full, LANE)]
        parts += [v[:, full:]] if full < m else []
        return parts[0] if len(parts) == 1 else jnp.concatenate(parts, axis=1)

    def half(j, n):
        return slice(j * T + n * TH, j * T + (n + 1) * TH)

    def quad(r0, rows, i):
        return slice(r0 + i // 2 * D2, r0 + i // 2 * D2 + rows)

    moments = {}

    def note(j, n, v):
        st = moments.setdefault((j, n), [v[0:1], None, None])
        for r in range(0, v.shape[0], 8):
            d = v[r:r + 8] - st[0]
            st[1] = d if st[1] is None else st[1] + d
            st[2] = d * d if st[2] is None else st[2] + d * d

    def layernorm(j, src, twice=False):
        stats = []

        def merge():
            low = lax.broadcasted_iota(jnp.int32, (8, TH), 0) < 4
            (c0, p0, q0), (c1, p1, q1) = moments.pop((j, 0)), moments.pop((j, 1))

            def average(u, v):
                return jnp.where(low, jnp.sum(u, axis=0, keepdims=True), jnp.sum(v, axis=0, keepdims=True)) * (1.0 / D)
            d = average(p0, p1)
            var = jnp.maximum(average(q0, q1) - d * d, 0.0)
            mean = jnp.where(low, c0, c1) + d
            r = lax.rsqrt(var + EPS)
            if twice:
                for n in range(2):
                    stat_ref[0:1, half(j, n)] = mean[4 * n:4 * n + 1]
                    stat_ref[1:2, half(j, n)] = r[4 * n:4 * n + 1]
                r = r * lax.rsqrt(var * r * r + EPS)
            stats.extend((mean[4 * n:4 * n + 1], r[4 * n:4 * n + 1]) for n in range(2))

        def apply(r0, t, gate):
            if not stats:
                merge()
            cs = slice(t, t + LANE)
            mean = [after(jnp.broadcast_to(stats[n][0][:, cs], (8, LANE)), gate) for n in range(2)]
            scale = [jnp.broadcast_to(stats[n][1][:, cs], (8, LANE)) for n in range(2)]
            blocks = []
            for i in range(4):
                c0 = half(j, i % 2).start + t
                v = src[quad(r0, 32, i), c0:c0 + LANE].reshape(4, 8, LANE)
                blocks.append(((v - mean[i % 2]) * scale[i % 2]).reshape(32, LANE))
            _put_rhs(b_d.at[j], r0, cs, *blocks)

        return [lambda gate, r0=r0, t=t: apply(r0, t, gate) for t in range(0, TH, LANE) for r0 in range(0, D2, 32)]

    def widen_input(j):
        for n in range(2):
            for r0 in range(0, D, GRP):
                x = io_buf[r0:r0 + GRP, half(j, n)].astype(f32)
                x_ref[r0:r0 + GRP, half(j, n)] = x
                note(j, n, x)

    def qkv(j, paced):
        def put(r0, i, val):
            kind, cs = r0 // D2, half(j, i % 2)
            for hl in range(4):
                h, r = 4 * (r0 % D2 // GRP + i // 2 * 2) + hl, _win_start(hl)
                win = val[r:r + WIN]
                if kind == 0:
                    k_ref[h, _words(cs.start, TH), :] = _pack(win.T)
                elif kind == 1:
                    q_ref[h, :, cs] = _pack(jnp.where(_own_rows(hl, TH), win * QSCALE, 0.0))
                else:
                    v_ref[h, :, cs] = _pack(jnp.where(_own_rows(hl, TH), win, 1.0))
        _matmul(a_qkv, b_d.at[j], GRP, put, paced=paced)

    def scores(h, j, c, m, side=()):
        s = _dot(_unpack(k_ref[h, _words(c * C, C), :]), _unpack(q_ref[h, :, j * W:(j + 1) * W]))
        s_ref[j % 2][c * C:(c + 1) * C, :] = s
        for i, f in enumerate(side):
            r = C * i // len(side) // 8 * 8
            f(s[r:r + 8, 0:LANE])
        top = jnp.max(s.reshape(C // 8, 8, W), axis=0)
        return top if m is None else jnp.maximum(m, top)

    def unit(h, j, top, side=()):
        ahead = [(h + (j + k) // NW, (j + k) % NW) for k in (1, 2)]
        ahead = [None if isinstance(a[0], int) and a[0] >= H else a for a in ahead]
        live = {}

        def step(c, gate):
            if c == 0:
                live['max'] = jnp.broadcast_to(jnp.max(top[0], axis=0, keepdims=True), (8, W))
                top[0], top[1] = top[1], None
            if c + 1 < NC and ahead[0]:
                top[0] = scores(*ahead[0], c + 1, top[0], side[c * len(side) // (NC - 1):(c + 1) * len(side) // (NC - 1)])
            s = s_ref[j % 2][c * C:(c + 1) * C, :].reshape(C // 8, 8, W)
            p = jnp.exp2(s - after(live['max'], gate)).reshape(C, W).astype(bf16)
            o = _dot(_unpack(v_ref[h, :, c * C:(c + 1) * C]), p)
            live['acc'] = o if c == 0 else live['acc'] + o
            if c + 1 == NC:
                if ahead[1]:
                    top[1] = scores(*ahead[1], 0, None)
                acc = live['acc']
                if isinstance(h, int):
                    total = acc[0:1] if h % 2 else acc[WIN - 1:WIN]
                else:
                    total = jnp.where(h % 2 == 0, acc[WIN - 1:WIN], acc[0:1])
                o_ref[h, :, j * W:(j + 1) * W] = acc * (1.0 / total)
        return [lambda gate=None, c=c: step(c, gate) for c in range(NC)]

    def attention_head_loop():
        top = [None, scores(0, 1, 0, None)]
        for c in range(NC):
            top[0] = scores(0, 0, c, top[0])

        def body(i, carry):
            carry = list(carry)
            for h in (2 * i, 2 * i + 1):
                for j in range(NW):
                    for step in unit(h, j, carry):
                        step()
            return tuple(carry)
        return list(lax.fori_loop(0, H // 2 - 1, body, tuple(top)))

    def o_operands(j, i):
        _put_rhs(b_o.at[j], i * WIN, slice(None),
                 *[o_ref[i + n // 2 * (H // 2), :, half(j, n % 2)] for n in range(4)])

    def wo(j, paced):
        def add(r0, i, val):
            at = quad(r0, D2, i), half(j, i % 2)
            x = x_ref[at] + val
            x_ref[at] = x
            note(j, i % 2, x)
        _matmul(a_o, b_o.at[j], D2, add, paced=paced)

    def w1(j, paced):
        def act(r0, i, val):
            c0 = LANE + half(j, i % 2).start
            h_ref[quad(r0, GRP, i), c0:c0 + TH] = _gelu(val)
        _matmul(a_1, b_d.at[j], GRP, act, paced=paced)

    def shift(j):
        def shifted(rows, n):
            by = SHIFTS[rows.start // GRP]
            lo = half(j, n).start + (0 if by > 0 else LANE)
            off = LANE - by if by > 0 else -by
            return h_ref[rows, lo:lo + TH + LANE][:, off:off + TH]
        for r0 in range(0, D2, 16):
            _put_rhs(b_d.at[j], r0, slice(None), *[shifted(quad(r0, 16, i), i % 2) for i in range(4)])

    def w2(j, paced):
        def add(r0, i, val):
            rows, cs = quad(r0, D2, i), half(j, i % 2)
            x1 = (x_ref[rows, cs] - stat_ref[0:1, cs]) * stat_ref[1:2, cs] + val
            y_ref[rows, cs] = x1
            note(j, i % 2, x1)
        _matmul(a_2, b_d.at[j], D2, add, paced=paced)

    def w3(j, paced):
        def staged(r0):
            return g_ref[(4 * j + (r0 + LANE) // HID) % 3]

        def act(r0, i, val):
            staged(r0)[i, 0:val.shape[0], :] = _gelu(val)

        def operands(r0, rows):
            def step(rr, t, i, gate):
                def quadrant(q):
                    return [staged(r0)[q, r:r + 16, c0:c0 + LANE] for r in range(rr, rows, LANE) for c0 in (t, t + TH // 2)]
                u, v, sign = ((0, None, 0), (2, 0, -1), (3, None, 0), (0, 3, 1), (2, 3, 1), (1, 3, -1), (0, 1, 1))[i]
                x = [after(part, gate) for part in quadrant(u)]
                if v is not None:
                    x = [a + b if sign > 0 else a - b for a, b in zip(x, quadrant(v))]
                if rows == LANE:
                    ops, dst = (x[0], None, None, x[0], None, x[1], x[0] + x[1]), FB
                else:
                    ops, dst = _rhs(*x), (r0 - LANE) // 2
                for k, op in enumerate(ops):
                    if op is not None:
                        b_f[j][i, k, _words(dst + rr, 16), t:t + LANE] = _pack_mixed(op)
            return [lambda gate, rr=rr, t=t, i=i: step(rr, t, i, gate)
                    for rr in range(0, LANE, 16) for t in range(0, TH // 2, LANE) for i in range(7)]
        return _matmul(a_3, b_d.at[j], HID, act, later=operands, paced=paced)

    def w4(j, last, paced):
        def add(r0, i, val):
            at = quad(r0, D2, i), half(j, i % 2)
            x = (x_ref[at] + y_ref[at]) + val
            if last:
                io_buf[at] = x.astype(bf16)
                out_copy(j, i).start()
            else:
                x_ref[at] = x
                note(j, i % 2, x)
        _matmul(a_4, b_f[j], D2, add, paced=paced)

    def transposed_halves(w_ref, cs, gate):
        return [_mixed(after(w_ref[r:r + D2, cs].astype(f32), gate)).T for r in (0, D2)]

    def prep_qkv(i, gate):
        c0 = (1, 0, 2)[i] * D
        lo = c0 // LANE * LANE
        wl, wr = transposed_halves(wqkv_in, slice(lo, min(pl.cdiv(c0 + D, LANE) * LANE, 3 * D)), gate)
        r = c0 - lo
        _put_lhs(a_qkv, i * D2, wl[r:r + D2], wr[r:r + D2], wl[r + D2:r + D], wr[r + D2:r + D])

    def prep_o(gate):
        halves = []
        for r in (0, D2):
            w = after(wo_in[r:r + D2, :].astype(f32), gate)
            wins = [jnp.where(_own_rows(h, D), w[_win_start(h):_win_start(h) + WIN], 0.0) for h in range(H // 2)]
            halves.append(_mixed(jnp.concatenate(wins, axis=0)).T)
        wl, wr = halves
        _put_lhs(a_o, 0, wl[0:D2], wr[0:D2], wl[D2:D], wr[D2:D])

    def prep_square(w_ref, a_ref, gate):
        wl, wr = transposed_halves(w_ref, slice(None), gate)
        _put_lhs(a_ref, 0, wl[0:D2], wr[0:D2], wl[D2:D], wr[D2:D])

    def prep_3(t, gate):
        blocks = [v for c0 in (t * LANE, F2 + t * LANE) for v in transposed_halves(w3_in, slice(c0, c0 + LANE), gate)]
        _put_lhs(a_3, (1, 3, 5, 0, 2, 4, 6)[t] * LANE, *[_unmixed(v) for v in blocks])

    def prep_4(r0, c0, gate):
        def part(q, c):
            return _lhs(*[after(w4_in[quad(q * GRP + r0, 16, i), i % 2 * F2 + c:i % 2 * F2 + c + LANE].astype(f32), gate)
                          for i in range(4)])
        y11, y21 = part(0, c0), part(1, c0)
        if c0 < FB:
            y12, y22 = part(0, FA + c0), part(1, FA + c0)
        for i in range(7):
            if c0 < FB:
                ops = _lhs(y11[i], y12[i], y21[i], y22[i])
            else:
                ops = (y21[i], None, None, y11[i], None, y11[i], y21[i] - y11[i])
            for k, op in enumerate(ops):
                if op is not None:
                    a_4[i, k, _words(r0, 16), c0:c0 + LANE] = _pack(op)

    def prep_rest():
        gap = [lambda gate: None] * 3
        steps = ([prep_o] + gap + [lambda gate: prep_square(w1_in, a_1, gate)] + gap
                 + [lambda gate: prep_square(w2_in, a_2, gate)] + gap)
        for t in range(F2 // LANE):
            steps += [lambda gate, t=t: prep_3(t, gate)] + gap[:2]
        return steps + [lambda gate, r0=r0, c0=c0: prep_4(r0, c0, gate)
                        for r0 in range(0, GRP, 16) for c0 in range(0, FA, LANE)]

    def rest_of_round(top, last, side):
        n = 2 * NW - 2
        units = [unit(H - 2 + u // NW, u % NW, top, side[u * len(side) // n:(u + 1) * len(side) // n] if u < n else ())
                 for u in range(2 * NW)]
        for u in range(2 * NW - 1):
            for step in units[u]:
                step()
            if u == NW - 1:
                for j in range(2):
                    for i in range(H // 2 - 1):
                        o_operands(j, i)
            if u == NW + 1:
                o_operands(0, H // 2 - 1)
        wo(0, [(units[-1], (0.0, 0.7))])
        o_operands(1, H // 2 - 1)
        span = (0.15, 0.7)
        wo(1, [(layernorm(0, x_ref, twice=True), span)])
        w1(0, [(layernorm(1, x_ref, twice=True), span)])
        w1(1, [])
        shift(0)
        shift(1)
        w2(0, [])
        w2(1, [(layernorm(0, y_ref), span)])
        fence()
        todo = w3(0, [(layernorm(1, y_ref), (0.02, 0.28))])
        todo = w3(1, [(todo, (0.0, 0.45))])
        w4(0, last, [(todo, (0.0, 0.45))])
        w4(1, last, [] if last else [(layernorm(0, x_ref), (0.05, 0.8))])

    x_cp[0].start()
    w_cp[0].start()
    fence()
    h_ref[:, 0:LANE] = jnp.zeros((D, LANE), f32)
    h_ref[:, LANE + S:] = jnp.zeros((D, LANE), f32)
    x_cp[0].wait()
    widen_input(0)
    for step in layernorm(0, x_ref):
        step(None)
    w_cp[0].wait()
    x_cp[1].start()
    prep_qkv(0, None)

    def second_block(gate):
        x_cp[1].wait()
        widen_input(1)
    qkv(0, [([second_block] + layernorm(1, x_ref), (0.4, 0.8)),
            ([lambda gate: prep_qkv(1, gate), lambda gate: prep_qkv(2, gate)], (0.02, 0.4))])
    qkv(1, [])
    for cp in w_cp[1:]:
        cp.start()
    top = attention_head_loop()
    for cp in w_cp[1:]:
        cp.wait()
    rest_of_round(top, False, prep_rest())

    fence()
    qkv(0, [(layernorm(1, x_ref), (0.1, 0.8))])
    qkv(1, [])
    rest_of_round(attention_head_loop(), True, [])
    for j in range(2):
        for i in range(4):
            out_copy(j, i).wait()


@jax.jit
def pallas_interleave_layers__mha_block__mixer_s_mlp__prompt_kernel(
    A_x: jax.Array,
    A_wqkv: jax.Array,
    A_wo: jax.Array,
    B_x: jax.Array,
    B_w1: jax.Array,
    B_w2: jax.Array,
    B_w3: jax.Array,
    B_w4: jax.Array,
):
    del B_x
    in_hbm = pl.BlockSpec(memory_space=pl.ANY)
    out = pl.pallas_call(
        _kernel,
        out_shape=jax.ShapeDtypeStruct((D, S), bf16),
        in_specs=[in_hbm] * 7,
        out_specs=in_hbm,
        scratch_shapes=[
            pltpu.VMEM((D, S), bf16),
            pltpu.VMEM((D, 3 * D), bf16),
            pltpu.VMEM((D, D), bf16),
            pltpu.VMEM((D, D), bf16),
            pltpu.VMEM((D, D), bf16),
            pltpu.VMEM((D, F), bf16),
            pltpu.VMEM((D, F), bf16),
            pltpu.VMEM((7, 3 * D2 // 2, D2), u32),
            pltpu.VMEM((7, D2 // 2, H * WIN // 2), u32),
            pltpu.VMEM((7, D2 // 2, D2), u32),
            pltpu.VMEM((7, D2 // 2, D2), u32),
            pltpu.VMEM((7, F2 // 2, D2), u32),
            pltpu.VMEM((7, 7, GRP // 2, FA), u32),
            pltpu.VMEM((2, 7, D2 // 2, TH), u32),
            pltpu.VMEM((2, 7, H * WIN // 4, TH), u32),
            pltpu.VMEM((7, 7, FA // 2, TH // 2), u32),
            pltpu.VMEM((7, 7, FA // 2, TH // 2), u32),
            pltpu.VMEM((4, HID, TH), f32),
            pltpu.VMEM((4, HID, TH), f32),
            pltpu.VMEM((4, HID, TH), f32),
            pltpu.VMEM((2, 8, LANE), f32),
            pltpu.VMEM((8, S), f32),
            pltpu.VMEM((D, S), f32),
            pltpu.VMEM((D, S), f32),
            pltpu.VMEM((H, WIN // 2, S), u32),
            pltpu.VMEM((H, S // 2, WIN), u32),
            pltpu.VMEM((H, WIN // 2, S), u32),
            pltpu.VMEM((H, WIN, S), f32),
            pltpu.VMEM((S, W), f32),
            pltpu.VMEM((S, W), f32),
            pltpu.VMEM((D, S + 2 * LANE), f32),
            pltpu.SemaphoreType.DMA((8,)),
            pltpu.SemaphoreType.DMA((8,)),
        ],
        compiler_params=pltpu.CompilerParams(vmem_limit_bytes=124 * 2 ** 20),
        name='fused',
    )(A_x[0].T, A_wqkv, A_wo, B_w1, B_w2, B_w3, B_w4.T)
    return out.T[None]
```

```python
import math

import jax
import jax.numpy as jnp
from jax import lax
import jax.experimental.pallas as pl
import jax.experimental.pallas.tpu as pltpu

f32, bf16, u32 = jnp.float32, jnp.bfloat16, jnp.uint32

S, D, H, F = 2048, 448, 16, 1792
DH = D // H
D2, F2 = D // 2, F // 2
GRP = 4 * DH
WIN = 32
LANE = 128
EPS = 1e-5
QSCALE = DH ** -0.5 * math.log2(math.e)
GELU_C = math.sqrt(2.0 / math.pi)
SHIFTS = (1, -1, 2, -2)

T = 1024
TH = T // 2
W = 512
NW = S // W
C = 128
NC = S // C
HID = 256
FA, FB = 512, 384
DEPTH = (FA, FB, FB, FA, FB, FA, FA)


def _dot(a, b):
    return jnp.dot(a, b, preferred_element_type=f32)


def _pack(v):
    return pltpu.bitcast(v.astype(bf16), u32)


def _pack_mixed(v):
    n, m = v.shape
    v = v.reshape(n // 16, 2, 8, m)
    return pltpu.pack_elementwise([v[:, 0].reshape(n // 2, m), v[:, 1].reshape(n // 2, m)], packed_dtype=bf16)


def _unpack(w):
    return pltpu.bitcast(w, bf16)


def _mixed(w):
    return _unpack(_pack_mixed(w)).astype(f32)


def _unmixed(w):
    n, m = w.shape
    words = pltpu.bitcast(w.astype(bf16), u32)
    parts = [pltpu.unpack_elementwise(words, index=i, packed_dtype=bf16, unpacked_dtype=f32).reshape(n // 16, 1, 8, m)
             for i in range(2)]
    return jnp.concatenate(parts, axis=1).reshape(n, m)


def _words(r0, n):
    return slice(r0 // 2, (r0 + n) // 2)


def _gelu(x):
    hx = 0.5 * x
    return hx * jnp.tanh(x * (x * x * (GELU_C * 0.044715) + GELU_C)) + hx


def _win_start(h):
    return (DH * h) // 8 * 8


def _own_rows(h, width):
    r = lax.broadcasted_iota(jnp.int32, (WIN, width), 0)
    off = DH * h - _win_start(h)
    return (r >= off) & (r < off + DH)


def _lhs(a11, a12, a21, a22):
    return a21 + a22, a22, a11 + a12, a11 + a22, a12 - a22, a11, a21 - a11


def _rhs(b11, b12, b21, b22):
    return b11, b21 - b11, b22, b11 + b22, b21 + b22, b12 - b22, b11 + b12


def _block(i, m):
    if i == 0:
        return (m[1] - m[2]) + m[3] + m[4]
    if i == 1:
        return m[5] + m[2]
    if i == 2:
        return m[0] + m[1]
    return (m[3] - m[0]) + m[5] + m[6]


def _put_lhs(a_ref, r0, *blocks):
    for i, v in enumerate(_lhs(*blocks)):
        a_ref[i, _words(r0, v.shape[0]), :] = _pack(v)


def _put_rhs(b_ref, r0, cols, *blocks):
    for i, v in enumerate(_rhs(*blocks)):
        b_ref[i, _words(r0, v.shape[0]), cols] = _pack_mixed(v)


def _matmul(a_ref, b_ref, chunk, now, later=None, paced=()):
    twice = len(a_ref.shape) == 4
    total = 4 * a_ref.shape[2] if twice else 2 * a_ref.shape[1]
    due, todo = {}, []
    for funcs, (begin, end) in paced:
        for k, f in enumerate(funcs):
            due.setdefault(int(total * 7 // 8 * (begin + (end - begin) * k / len(funcs))), []).append(f)
    starts = [0] + list(range(total % chunk or chunk, total + 1, chunk))
    for r0, r1 in zip(starts, starts[1:]):
        rows, m = r1 - r0, []
        for k, f in enumerate(todo):
            due.setdefault((r0 * 7 + rows * 7 * k // len(todo)) // 8, []).append(f)
        for i in range(7):
            if twice:
                p = [_dot(_unpack(a_ref[i, k, :, 0:n]), _unpack(b_ref[i, k, 0:n // 2, :])) for k, n in enumerate(DEPTH)]
                c = [_block(k, p) for k in range(4)]
                m.append(jnp.concatenate([jnp.concatenate(c[0:2], axis=1), jnp.concatenate(c[2:4], axis=1)], axis=0))
            else:
                m.append(_dot(_unpack(a_ref[i, _words(r0, rows), :]), _unpack(b_ref[i])))
            for r in range(0, rows, 8):
                for f in due.get((r0 * 7 + i * rows + r) // 8, ()):
                    f(p[r // 32][r % 32 * 3:r % 32 * 3 + 8, 0:LANE] if twice else m[i][r:r + 8, 0:LANE])
            done = {1: 2, 4: 0, 5: 1, 6: 3}.get(i)
            if done is not None:
                now(r0, done, _block(done, m))
        todo = later(r0, rows) if later is not None else []
    return todo


def _kernel(x_hbm, wqkv_hbm, wo_hbm, w1_hbm, w2_hbm, w3_hbm, w4_hbm, out_hbm,
            io_buf, wqkv_in, wo_in, w1_in, w2_in, w3_in, w4_in,
            a_qkv, a_o, a_1, a_2, a_3, a_4,
            b_d, b_o, b_f0, b_f1, g_ref0, g_ref1, g_ref2, one_ref, stat_ref,
            x_ref, y_ref, q_ref, k_ref, v_ref, o_ref, s_ref0, s_ref1, h_ref,
            in_sem, out_sem):
    b_f, g_ref, s_ref = (b_f0, b_f1), (g_ref0, g_ref1, g_ref2), (s_ref0, s_ref1)

    x_cp = [pltpu.make_async_copy(x_hbm.at[:, pl.ds(j * T, T)], io_buf.at[:, pl.ds(j * T, T)], in_sem.at[6 + j])
            for j in range(2)]
    qkv_cp = [pltpu.make_async_copy(wqkv_hbm.at[:, pl.ds(c0, n)], wqkv_in.at[:, pl.ds(c0, n)], in_sem.at[8 + i])
              for i, (c0, n) in enumerate(((384, 512), (0, 384), (896, D)))]
    w_cp = [pltpu.make_async_copy(src, dst, in_sem.at[i]) for i, (src, dst) in enumerate((
        (wo_hbm, wo_in), (w1_hbm, w1_in), (w2_hbm, w2_in), (w3_hbm, w3_in), (w4_hbm, w4_in)))]

    def out_copy(j, i):
        at = (pl.ds(i // 2 * D2, D2), pl.ds(j * T + i % 2 * TH, TH))
        return pltpu.make_async_copy(io_buf.at[at], out_hbm.at[at], out_sem.at[4 * j + i])

    def fence():
        def body(i, carry):
            one_ref[i] = jnp.ones((8, LANE), f32)
            return carry
        lax.fori_loop(0, 2, body, 0)

    def after(v, gate):
        if gate is None:
            return v
        n, m = v.shape
        full = m // LANE * LANE
        parts = [jnp.where(one_ref[0] > 0.0, v[:, t:t + LANE].reshape(n // 8, 8, LANE), gate).reshape(n, LANE)
                 for t in range(0, full, LANE)]
        parts += [v[:, full:]] if full < m else []
        return parts[0] if len(parts) == 1 else jnp.concatenate(parts, axis=1)

    def half(j, n):
        return slice(j * T + n * TH, j * T + (n + 1) * TH)

    def quad(r0, rows, i):
        return slice(r0 + i // 2 * D2, r0 + i // 2 * D2 + rows)

    moments = {}

    def note(j, n, v):
        st = moments.setdefault((j, n), [v[0:1], None, None])
        for r in range(0, v.shape[0], 8):
            d = v[r:r + 8] - st[0]
            st[1] = d if st[1] is None else st[1] + d
            st[2] = d * d if st[2] is None else st[2] + d * d

    def layernorm(j, src, twice=False):
        stats = []

        def merge():
            low = lax.broadcasted_iota(jnp.int32, (8, TH), 0) < 4
            (c0, p0, q0), (c1, p1, q1) = moments.pop((j, 0)), moments.pop((j, 1))

            def average(u, v):
                return jnp.where(low, jnp.sum(u, axis=0, keepdims=True), jnp.sum(v, axis=0, keepdims=True)) * (1.0 / D)
            d = average(p0, p1)
            var = jnp.maximum(average(q0, q1) - d * d, 0.0)
            mean = jnp.where(low, c0, c1) + d
            r = lax.rsqrt(var + EPS)
            if twice:
                for n in range(2):
                    stat_ref[0:1, half(j, n)] = mean[4 * n:4 * n + 1]
                    stat_ref[1:2, half(j, n)] = r[4 * n:4 * n + 1]
                r = r * lax.rsqrt(var * r * r + EPS)
            stats.extend((mean[4 * n:4 * n + 1], r[4 * n:4 * n + 1]) for n in range(2))

        def apply(r0, t, gate):
            if not stats:
                merge()
            cs = slice(t, t + LANE)
            mean = [after(jnp.broadcast_to(stats[n][0][:, cs], (8, LANE)), gate) for n in range(2)]
            scale = [jnp.broadcast_to(stats[n][1][:, cs], (8, LANE)) for n in range(2)]
            blocks = []
            for i in range(4):
                c0 = half(j, i % 2).start + t
                v = src[quad(r0, 16, i), c0:c0 + LANE].reshape(2, 8, LANE)
                blocks.append(((v - mean[i % 2]) * scale[i % 2]).reshape(16, LANE))
            _put_rhs(b_d.at[j], r0, cs, *blocks)

        return [lambda gate, r0=r0, t=t: apply(r0, t, gate) for t in range(0, TH, LANE) for r0 in range(0, D2, 16)]

    def widen_input(j):
        for n in range(2):
            for r0 in range(0, D, GRP):
                x = io_buf[r0:r0 + GRP, half(j, n)].astype(f32)
                x_ref[r0:r0 + GRP, half(j, n)] = x
                note(j, n, x)

    def qkv(j, paced):
        def put(r0, i, val):
            kind, cs = r0 // D2, half(j, i % 2)
            for hl in range(4):
                h, r = 4 * (r0 % D2 // GRP + i // 2 * 2) + hl, _win_start(hl)
                win = val[r:r + WIN]
                if kind == 0:
                    k_ref[h, _words(cs.start, TH), :] = _pack(win.T)
                elif kind == 1:
                    q_ref[h * NW + 2 * j + i % 2] = _pack(jnp.where(_own_rows(hl, TH), win * QSCALE, 0.0))
                else:
                    v_ref[h, :, cs] = _pack(jnp.where(_own_rows(hl, TH), win, 1.0))
        _matmul(a_qkv, b_d.at[j], GRP, put, paced=paced)

    def scores(h, j, c, m, side=()):
        s = _dot(_unpack(k_ref[h, _words(c * C, C), :]), _unpack(q_ref[h * NW + j]))
        s_ref[j % 2][c * C:(c + 1) * C, :] = s
        for i, f in enumerate(side):
            r = C * i // len(side) // 8 * 8
            f(s[r:r + 8, 0:LANE])
        top = jnp.max(s.reshape(C // 8, 8, W), axis=0)
        return top if m is None else jnp.maximum(m, top)

    def unit(pair, u, top, left=2, side=()):
        live = {}

        def place(k):
            return 2 * pair + (u + k) // NW, (u + k) % NW

        def step(c, gate):
            h, j = place(0)
            if c == 0:
                live['max'] = jnp.broadcast_to(jnp.max(top[0], axis=0, keepdims=True), (8, W))
                top[0], top[1] = top[1], None
            if c + 1 < NC and left >= 1:
                top[0] = scores(*place(1), c + 1, top[0], side[c * len(side) // (NC - 1):(c + 1) * len(side) // (NC - 1)])
            s = s_ref[j % 2][c * C:(c + 1) * C, :].reshape(C // 8, 8, W)
            p = jnp.exp2(s - after(live['max'], gate)).reshape(C, W).astype(bf16)
            o = _dot(_unpack(v_ref[h, :, c * C:(c + 1) * C]), p)
            live['acc'] = o if c == 0 else live['acc'] + o
            if c + 1 == NC:
                if left >= 2:
                    top[1] = scores(*place(2), 0, None)
                acc = live['acc']
                o_ref[h * NW + j] = acc * (1.0 / (acc[0:1] if u // NW else acc[WIN - 1:WIN]))
        return [lambda gate=None, c=c: step(c, gate) for c in range(NC)]

    def attention_loop():
        top = [None, scores(0, 1, 0, None)]
        for c in range(NC):
            top[0] = scores(0, 0, c, top[0])

        def body(pair, carry):
            carry = list(carry)
            for u in range(2 * NW):
                for step in unit(pair, u, carry):
                    step()
            return tuple(carry)
        return list(lax.fori_loop(0, H // 2 - 1, body, tuple(top)))

    def o_operands(j, i):
        _put_rhs(b_o.at[j], i * WIN, slice(None), *[o_ref[(i + n // 2 * (H // 2)) * NW + 2 * j + n % 2] for n in range(4)])

    def wo(j, paced):
        def add(r0, i, val):
            at = quad(r0, D2, i), half(j, i % 2)
            x = x_ref[at] + val
            x_ref[at] = x
            note(j, i % 2, x)
        _matmul(a_o, b_o.at[j], D2, add, paced=paced)

    def w1(j, paced):
        def act(r0, i, val):
            c0 = LANE + half(j, i % 2).start
            h_ref[quad(r0, GRP, i), c0:c0 + TH] = _gelu(val)
        _matmul(a_1, b_d.at[j], GRP, act, paced=paced)

    def shift(j):
        def shifted(rows, n):
            by = SHIFTS[rows.start // GRP]
            lo = half(j, n).start + (0 if by > 0 else LANE)
            off = LANE - by if by > 0 else -by
            return h_ref[rows, lo:lo + TH + LANE][:, off:off + TH]
        for r0 in range(0, D2, 16):
            _put_rhs(b_d.at[j], r0, slice(None), *[shifted(quad(r0, 16, i), i % 2) for i in range(4)])

    def w2(j, paced):
        def add(r0, i, val):
            rows, cs = quad(r0, D2, i), half(j, i % 2)
            x1 = (x_ref[rows, cs] - stat_ref[0:1, cs]) * stat_ref[1:2, cs] + val
            y_ref[rows, cs] = x1
            note(j, i % 2, x1)
        _matmul(a_2, b_d.at[j], D2, add, paced=paced)

    def w3(j, paced):
        def staged(r0):
            return g_ref[(4 * j + (r0 + LANE) // HID) % 3]

        def act(r0, i, val):
            staged(r0)[i, 0:val.shape[0], :] = _gelu(val)

        def operands(r0, rows):
            def step(rr, t, i, gate):
                def quadrant(q):
                    return [staged(r0)[q, r:r + 16, c0:c0 + LANE] for r in range(rr, rows, LANE) for c0 in (t, t + TH // 2)]
                u, v, sign = ((0, None, 0), (2, 0, -1), (3, None, 0), (0, 3, 1), (2, 3, 1), (1, 3, -1), (0, 1, 1))[i]
                x = [after(part, gate) for part in quadrant(u)]
                if v is not None:
                    x = [a + b if sign > 0 else a - b for a, b in zip(x, quadrant(v))]
                if rows == LANE:
                    ops, dst = (x[0], None, None, x[0], None, x[1], x[0] + x[1]), FB
                else:
                    ops, dst = _rhs(*x), (r0 - LANE) // 2
                for k, op in enumerate(ops):
                    if op is not None:
                        b_f[j][i, k, _words(dst + rr, 16), t:t + LANE] = _pack_mixed(op)
            return [lambda gate, rr=rr, t=t, i=i: step(rr, t, i, gate)
                    for rr in range(0, LANE, 16) for t in range(0, TH // 2, LANE) for i in range(7)]
        return _matmul(a_3, b_d.at[j], HID, act, later=operands, paced=paced)

    def w4(j, last, paced):
        def add(r0, i, val):
            at = quad(r0, D2, i), half(j, i % 2)
            x = (x_ref[at] + y_ref[at]) + val
            if last:
                io_buf[at] = x.astype(bf16)
                out_copy(j, i).start()
            else:
                x_ref[at] = x
                note(j, i % 2, x)
        _matmul(a_4, b_f[j], D2, add, paced=paced)

    def transposed_halves(w_ref, cs, gate):
        return [_mixed(after(w_ref[r:r + D2, cs].astype(f32), gate)).T for r in (0, D2)]

    def prep_qkv(i, gate):
        qkv_cp[i].wait()
        c0 = (1, 0, 2)[i] * D
        lo = c0 // LANE * LANE
        wl, wr = transposed_halves(wqkv_in, slice(lo, min(pl.cdiv(c0 + D, LANE) * LANE, 3 * D)), gate)
        r = c0 - lo
        _put_lhs(a_qkv, i * D2, wl[r:r + D2], wr[r:r + D2], wl[r + D2:r + D], wr[r + D2:r + D])

    def prep_o(gate):
        halves = []
        for r in (0, D2):
            w = after(wo_in[r:r + D2, :].astype(f32), gate)
            wins = [jnp.where(_own_rows(h, D), w[_win_start(h):_win_start(h) + WIN], 0.0) for h in range(H // 2)]
            halves.append(_mixed(jnp.concatenate(wins, axis=0)).T)
        wl, wr = halves
        _put_lhs(a_o, 0, wl[0:D2], wr[0:D2], wl[D2:D], wr[D2:D])

    def prep_square(w_ref, a_ref, gate):
        wl, wr = transposed_halves(w_ref, slice(None), gate)
        _put_lhs(a_ref, 0, wl[0:D2], wr[0:D2], wl[D2:D], wr[D2:D])

    def prep_3(t, gate):
        blocks = [v for c0 in (t * LANE, F2 + t * LANE) for v in transposed_halves(w3_in, slice(c0, c0 + LANE), gate)]
        _put_lhs(a_3, (1, 3, 5, 0, 2, 4, 6)[t] * LANE, *[_unmixed(v) for v in blocks])

    def prep_4(r0, c0, i, gate):
        def part(q, c):
            def blk(n):
                return _unmixed(w4_in[quad(q * GRP + r0, 16, n), n % 2 * F2 + c:n % 2 * F2 + c + LANE])
            u, v, sign = ((2, 3, 1), (3, None, 0), (0, 1, 1), (0, 3, 1), (1, 3, -1), (0, None, 0), (2, 0, -1))[i]
            y = after(blk(u), gate)
            return y if v is None else y + blk(v) if sign > 0 else y - blk(v)
        y11, y21 = part(0, c0), part(1, c0)
        if c0 < FB:
            ops = _lhs(y11, part(0, FA + c0), y21, part(1, FA + c0))
        else:
            ops = (y21, None, None, y11, None, y11, y21 - y11)
        for k, op in enumerate(ops):
            if op is not None:
                a_4[i, k, _words(r0, 16), c0:c0 + LANE] = _pack_mixed(op)

    def prep_rest():
        gap = [lambda gate: None] * 15
        steps = ([prep_o] + gap * 2 + [lambda gate: prep_square(w1_in, a_1, gate)] + gap * 2
                 + [lambda gate: prep_square(w2_in, a_2, gate)] + gap * 2)
        for t in range(F2 // LANE):
            steps += [lambda gate, t=t: prep_3(t, gate)] + gap
        return steps + [lambda gate, r0=r0, c0=c0, i=i: prep_4(r0, c0, i, gate)
                        for r0 in range(0, GRP, 16) for c0 in range(0, FA, LANE) for i in range(7)]

    def rest_of_round(top, last, side):
        n = 2 * NW - 2
        units = [unit(H // 2 - 1, u, top, 2 * NW - 1 - u, side[u * len(side) // n:(u + 1) * len(side) // n])
                 for u in range(2 * NW)]
        for u in range(2 * NW - 1):
            for step in units[u]:
                step()
            if u == NW:
                for j in range(2):
                    for i in range(H // 2 - 1):
                        o_operands(j, i)
            if u == NW + 1:
                o_operands(0, H // 2 - 1)
        wo(0, [(units[-1], (0.0, 0.7))])
        o_operands(1, H // 2 - 1)
        span = (0.05, 0.7)
        wo(1, [(layernorm(0, x_ref, twice=True), span)])
        w1(0, [(layernorm(1, x_ref, twice=True), span)])
        w1(1, [])
        shift(0)
        shift(1)
        w2(0, [])
        w2(1, [(layernorm(0, y_ref), span)])
        fence()
        todo = w3(0, [(layernorm(1, y_ref), (0.02, 0.28))])
        todo = w3(1, [(todo, (0.0, 0.45))])
        w4(0, last, [(todo, (0.0, 0.45))])
        w4(1, last, [] if last else [(layernorm(0, x_ref), (0.05, 0.8))])

    qkv_cp[0].start()
    x_cp[0].start()
    fence()
    h_ref[:, 0:LANE] = jnp.zeros((D, LANE), f32)
    h_ref[:, LANE + S:] = jnp.zeros((D, LANE), f32)
    prep_qkv(0, None)
    x_cp[0].wait()
    for cp in (qkv_cp[1], qkv_cp[2], x_cp[1]):
        cp.start()
    widen_input(0)
    for step in layernorm(0, x_ref):
        step(None)

    def arrivals(gate):
        x_cp[1].wait()
        prep_qkv(2, gate)
        widen_input(1)
    qkv(0, [([lambda gate: prep_qkv(1, gate), arrivals], (0.15, 0.85)), (layernorm(1, x_ref), (0.6, 0.92))])
    qkv(1, [])
    for cp in w_cp:
        cp.start()
    top = attention_loop()
    for cp in w_cp:
        cp.wait()
    rest_of_round(top, False, prep_rest())

    fence()
    qkv(0, [(layernorm(1, x_ref), (0.1, 0.8))])
    qkv(1, [])
    rest_of_round(attention_loop(), True, [])
    for j in range(2):
        for i in range(4):
            out_copy(j, i).wait()


@jax.jit
def pallas_interleave_layers__mha_block__mixer_s_mlp__prompt_kernel(
    A_x: jax.Array,
    A_wqkv: jax.Array,
    A_wo: jax.Array,
    B_x: jax.Array,
    B_w1: jax.Array,
    B_w2: jax.Array,
    B_w3: jax.Array,
    B_w4: jax.Array,
):
    del B_x
    in_hbm = pl.BlockSpec(memory_space=pl.ANY)
    out = pl.pallas_call(
        _kernel,
        out_shape=jax.ShapeDtypeStruct((D, S), bf16),
        in_specs=[in_hbm] * 7,
        out_specs=in_hbm,
        scratch_shapes=[
            pltpu.VMEM((D, S), bf16),
            pltpu.VMEM((D, 3 * D), bf16),
            pltpu.VMEM((D, D), bf16),
            pltpu.VMEM((D, D), bf16),
            pltpu.VMEM((D, D), bf16),
            pltpu.VMEM((D, F), bf16),
            pltpu.VMEM((D, F), bf16),
            pltpu.VMEM((7, 3 * D2 // 2, D2), u32),
            pltpu.VMEM((7, D2 // 2, H * WIN // 2), u32),
            pltpu.VMEM((7, D2 // 2, D2), u32),
            pltpu.VMEM((7, D2 // 2, D2), u32),
            pltpu.VMEM((7, F2 // 2, D2), u32),
            pltpu.VMEM((7, 7, GRP // 2, FA), u32),
            pltpu.VMEM((2, 7, D2 // 2, TH), u32),
            pltpu.VMEM((2, 7, H * WIN // 4, TH), u32),
            pltpu.VMEM((7, 7, FA // 2, TH // 2), u32),
            pltpu.VMEM((7, 7, FA // 2, TH // 2), u32),
            pltpu.VMEM((4, HID, TH), f32),
            pltpu.VMEM((4, HID, TH), f32),
            pltpu.VMEM((4, HID, TH), f32),
            pltpu.VMEM((2, 8, LANE), f32),
            pltpu.VMEM((8, S), f32),
            pltpu.VMEM((D, S), f32),
            pltpu.VMEM((D, S), f32),
            pltpu.VMEM((H * NW, WIN // 2, W), u32),
            pltpu.VMEM((H, S // 2, WIN), u32),
            pltpu.VMEM((H, WIN // 2, S), u32),
            pltpu.VMEM((H * NW, WIN, W), f32),
            pltpu.VMEM((S, W), f32),
            pltpu.VMEM((S, W), f32),
            pltpu.VMEM((D, S + 2 * LANE), f32),
            pltpu.SemaphoreType.DMA((11,)),
            pltpu.SemaphoreType.DMA((8,)),
        ],
        compiler_params=pltpu.CompilerParams(vmem_limit_bytes=124 * 2 ** 20),
        name='fused',
    )(A_x[0].T, A_wqkv, A_wo, B_w1, B_w2, B_w3, B_w4.T)
    return out.T[None]
```

```python
import math

import jax
import jax.numpy as jnp
from jax import lax
import jax.experimental.pallas as pl
import jax.experimental.pallas.tpu as pltpu

f32, bf16, u32 = jnp.float32, jnp.bfloat16, jnp.uint32

S, D, H, F = 2048, 448, 16, 1792
DH = D // H
D2, F2 = D // 2, F // 2
GRP = 4 * DH
WIN = 32
LANE = 128
EPS = 1e-5
QSCALE = DH ** -0.5 * math.log2(math.e)
GELU_C = math.sqrt(2.0 / math.pi)
SHIFTS = (1, -1, 2, -2)

T = 1024
TH = T // 2
W = 512
NW = S // W
C = 128
NC = S // C
HID = 256
FA, FB = 512, 384
DEPTH = (FA, FB, FB, FA, FB, FA, FA)


def _dot(a, b):
    return jnp.dot(a, b, preferred_element_type=f32)


def _put(ref, at, r0, c0, v):
    n, m = v.shape
    for t in range(0, m, LANE):
        part = v[:, t:t + LANE]
        ref[(*at, (c0 + t) // LANE, slice(r0, r0 + n), slice(0, part.shape[1]))] = part.astype(bf16)


def _get(ref, at, r0, n, c0, m):
    words = ref.bitcast(u32)
    parts = [pltpu.bitcast(words[(*at, (c0 + t) // LANE, _words(r0, n), slice(0, min(LANE, m - t)))], bf16)
             for t in range(0, m, LANE)]
    return parts[0] if len(parts) == 1 else jnp.concatenate(parts, axis=1)


def _words(r0, n):
    return slice(r0 // 2, (r0 + n) // 2)


def _gelu(x):
    hx = 0.5 * x
    return hx * jnp.tanh(x * (x * x * (GELU_C * 0.044715) + GELU_C)) + hx


def _win_start(h):
    return (DH * h) // 8 * 8


def _own_rows(h, width):
    r = lax.broadcasted_iota(jnp.int32, (WIN, width), 0)
    off = DH * h - _win_start(h)
    return (r >= off) & (r < off + DH)


def _lhs(a11, a12, a21, a22):
    return a21 + a22, a22, a11 + a12, a11 + a22, a12 - a22, a11, a21 - a11


def _rhs(b11, b12, b21, b22):
    return b11, b21 - b11, b22, b11 + b22, b21 + b22, b12 - b22, b11 + b12


def _block(i, m):
    if i == 0:
        return (m[1] - m[2]) + m[3] + m[4]
    if i == 1:
        return m[5] + m[2]
    if i == 2:
        return m[0] + m[1]
    return (m[3] - m[0]) + m[5] + m[6]


def _put_lhs(a_ref, r0, *blocks):
    for i, v in enumerate(_lhs(*blocks)):
        _put(a_ref, (i,), r0, 0, v)


def _put_rhs(b_ref, j, r0, c0, *blocks):
    for i, v in enumerate(_rhs(*blocks)):
        _put(b_ref, (j, i), r0, c0, v)


def _matmul(a_ref, b_ref, j, chunk, now, later=None, paced=()):
    twice = len(a_ref.shape) == 5
    total = a_ref.shape[-2] * (2 if twice else 1)
    depth = b_ref.shape[-2]
    due, todo = {}, []
    for funcs, (begin, end) in paced:
        for k, f in enumerate(funcs):
            due.setdefault(int(total * 7 // 8 * (begin + (end - begin) * k / len(funcs))), []).append(f)
    starts = [0] + list(range(total % chunk or chunk, total + 1, chunk))
    for r0, r1 in zip(starts, starts[1:]):
        rows, m = r1 - r0, []
        for k, f in enumerate(todo):
            due.setdefault((r0 * 7 + rows * 7 * k // len(todo)) // 8, []).append(f)
        for i in range(7):
            if twice:
                p = [_dot(_get(a_ref, (i, k), 0, rows // 2, 0, n), _get(b_ref, (i, k), 0, n, 0, TH // 2))
                     for k, n in enumerate(DEPTH)]
                c = [_block(k, p) for k in range(4)]
                m.append(jnp.concatenate([jnp.concatenate(c[0:2], axis=1), jnp.concatenate(c[2:4], axis=1)], axis=0))
            else:
                m.append(_dot(_get(a_ref, (i,), r0, rows, 0, depth), _get(b_ref, (j, i), 0, depth, 0, TH)))
            for r in range(0, rows, 8):
                for f in due.get((r0 * 7 + i * rows + r) // 8, ()):
                    f(p[r // 32][r % 32 * 3:r % 32 * 3 + 8, 0:LANE] if twice else m[i][r:r + 8, 0:LANE])
            done = {1: 2, 4: 0, 5: 1, 6: 3}.get(i)
            if done is not None:
                now(r0, done, _block(done, m))
        todo = later(r0, rows) if later is not None else []
    return todo


def _kernel(x_hbm, wqkv_hbm, wo_hbm, w1_hbm, w2_hbm, w3_hbm, w4_hbm, out_hbm,
            io_buf, wqkv_in, wo_in, w1_in, w2_in, w3_in, w4_in,
            a_qkv, a_o, a_1, a_2, a_3, a_4,
            b_d, b_o, b_f0, b_f1, g_ref0, g_ref1, g_ref2, one_ref, stat_ref,
            x_ref, y_ref, q_ref, k_ref, v_ref, o_ref, s_ref0, s_ref1, h_ref,
            in_sem, out_sem):
    b_f, g_ref, s_ref = (b_f0, b_f1), (g_ref0, g_ref1, g_ref2), (s_ref0, s_ref1)

    x_cp = [pltpu.make_async_copy(x_hbm.at[:, pl.ds(j * T, T)], io_buf.at[:, pl.ds(j * T, T)], in_sem.at[5 + j])
            for j in range(2)]
    qkv_cp = [pltpu.make_async_copy(wqkv_hbm.at[:, pl.ds(c0, n)], wqkv_in.at[:, pl.ds(c0, n)], in_sem.at[7 + i])
              for i, (c0, n) in enumerate(((384, 512), (0, 384), (896, D)))]
    w_cp = [pltpu.make_async_copy(src, dst, in_sem.at[i]) for i, (src, dst) in enumerate((
        (wo_hbm, wo_in), (w1_hbm, w1_in), (w2_hbm, w2_in), (w3_hbm, w3_in), (w4_hbm, w4_in)))]

    def out_copy(j, i):
        at = (pl.ds(i // 2 * D2, D2), pl.ds(j * T + i % 2 * TH, TH))
        return pltpu.make_async_copy(io_buf.at[at], out_hbm.at[at], out_sem.at[4 * j + i])

    def fence():
        def body(i, carry):
            one_ref[i] = jnp.ones((8, LANE), f32)
            return carry
        lax.fori_loop(0, 2, body, 0)

    def after(v, gate):
        if gate is None:
            return v
        n, m = v.shape
        full = m // LANE * LANE
        parts = [jnp.where(one_ref[0] > 0.0, v[:, t:t + LANE].reshape(n // 8, 8, LANE), gate).reshape(n, LANE)
                 for t in range(0, full, LANE)]
        parts += [v[:, full:]] if full < m else []
        return parts[0] if len(parts) == 1 else jnp.concatenate(parts, axis=1)

    def half(j, n):
        return slice(j * T + n * TH, j * T + (n + 1) * TH)

    def quad(r0, rows, i):
        return slice(r0 + i // 2 * D2, r0 + i // 2 * D2 + rows)

    moments = {}

    def note(j, n, v):
        st = moments.setdefault((j, n), [v[0:1], None, None])
        for r in range(0, v.shape[0], 8):
            d = v[r:r + 8] - st[0]
            st[1] = d if st[1] is None else st[1] + d
            st[2] = d * d if st[2] is None else st[2] + d * d

    def layernorm(j, src, twice=False):
        stats = []

        def merge():
            low = lax.broadcasted_iota(jnp.int32, (8, TH), 0) < 4
            (c0, p0, q0), (c1, p1, q1) = moments.pop((j, 0)), moments.pop((j, 1))

            def average(u, v):
                return jnp.where(low, jnp.sum(u, axis=0, keepdims=True), jnp.sum(v, axis=0, keepdims=True)) * (1.0 / D)
            d = average(p0, p1)
            var = jnp.maximum(average(q0, q1) - d * d, 0.0)
            mean = jnp.where(low, c0, c1) + d
            r = lax.rsqrt(var + EPS)
            if twice:
                for n in range(2):
                    stat_ref[0:1, half(j, n)] = mean[4 * n:4 * n + 1]
                    stat_ref[1:2, half(j, n)] = r[4 * n:4 * n + 1]
                r = r * lax.rsqrt(var * r * r + EPS)
            stats.extend((mean[4 * n:4 * n + 1], r[4 * n:4 * n + 1]) for n in range(2))

        def apply(r0, t, gate):
            if not stats:
                merge()
            cs = slice(t, t + 2 * LANE)
            mean = [after(jnp.broadcast_to(stats[n][0][:, cs], (8, 2 * LANE)), gate) for n in range(2)]
            scale = [jnp.broadcast_to(stats[n][1][:, cs], (8, 2 * LANE)) for n in range(2)]
            blocks = []
            for i in range(4):
                c0 = half(j, i % 2).start + t
                v = src[quad(r0, 16, i), c0:c0 + 2 * LANE].reshape(2, 8, 2 * LANE)
                blocks.append(((v - mean[i % 2]) * scale[i % 2]).reshape(16, 2 * LANE))
            _put_rhs(b_d, j, r0, t, *blocks)

        return [lambda gate, r0=r0, t=t: apply(r0, t, gate) for t in range(0, TH, 2 * LANE) for r0 in range(0, D2, 16)]

    def widen_input(j):
        for n in range(2):
            for r0 in range(0, D, GRP):
                x = io_buf[r0:r0 + GRP, half(j, n)].astype(f32)
                x_ref[r0:r0 + GRP, half(j, n)] = x
                note(j, n, x)

    def qkv(j, paced):
        def put(r0, i, val):
            kind, cs = r0 // D2, half(j, i % 2)
            for hl in range(4):
                h, r = 4 * (r0 % D2 // GRP + i // 2 * 2) + hl, _win_start(hl)
                win = val[r:r + WIN]
                if kind == 0:
                    _put(k_ref, (h,), cs.start, 0, win.T)
                elif kind == 1:
                    _put(q_ref, (h,), 0, cs.start, jnp.where(_own_rows(hl, TH), win * QSCALE, 0.0))
                else:
                    _put(v_ref, (h,), 0, cs.start, jnp.where(_own_rows(hl, TH), win, 1.0))
        _matmul(a_qkv, b_d, j, GRP, put, paced=paced)

    def scores(h, j, c, m, side=()):
        s = _dot(_get(k_ref, (h,), c * C, C, 0, WIN), _get(q_ref, (h,), 0, WIN, j * W, W))
        s_ref[j % 2][c * C:(c + 1) * C, :] = s
        for i, f in enumerate(side):
            r = C * i // len(side) // 8 * 8
            f(s[r:r + 8, 0:LANE])
        top = jnp.max(s.reshape(C // 8, 8, W), axis=0)
        return top if m is None else jnp.maximum(m, top)

    def unit(pair, u, top, left=2, side=()):
        live = {}

        def place(k):
            return 2 * pair + (u + k) // NW, (u + k) % NW

        def step(c, gate):
            h, j = place(0)
            if c == 0:
                live['max'] = jnp.broadcast_to(jnp.max(top[0], axis=0, keepdims=True), (8, W))
                top[0], top[1] = top[1], None
            if c + 1 < NC and left >= 1:
                top[0] = scores(*place(1), c + 1, top[0], side[c * len(side) // (NC - 1):(c + 1) * len(side) // (NC - 1)])
            s = s_ref[j % 2][c * C:(c + 1) * C, :].reshape(C // 8, 8, W)
            p = jnp.exp2(s - after(live['max'], gate)).reshape(C, W).astype(bf16)
            o = _dot(_get(v_ref, (h,), 0, WIN, c * C, C), p)
            live['acc'] = o if c == 0 else live['acc'] + o
            if c + 1 == NC:
                if left >= 2:
                    top[1] = scores(*place(2), 0, None)
                acc = live['acc']
                o_ref[h * NW + j] = acc * (1.0 / (acc[0:1] if u // NW else acc[WIN - 1:WIN]))
        return [lambda gate=None, c=c: step(c, gate) for c in range(NC)]

    def attention_loop():
        top = [None, scores(0, 1, 0, None)]
        for c in range(NC):
            top[0] = scores(0, 0, c, top[0])

        def body(pair, carry):
            carry = list(carry)
            for u in range(2 * NW):
                for step in unit(pair, u, carry):
                    step()
            return tuple(carry)
        return list(lax.fori_loop(0, H // 2 - 1, body, tuple(top)))

    def o_operands(j, i):
        _put_rhs(b_o, j, i * WIN, 0, *[o_ref[(i + n // 2 * (H // 2)) * NW + 2 * j + n % 2] for n in range(4)])

    def wo(j, paced):
        def add(r0, i, val):
            at = quad(r0, D2, i), half(j, i % 2)
            x = x_ref[at] + val
            x_ref[at] = x
            note(j, i % 2, x)
        _matmul(a_o, b_o, j, D2, add, paced=paced)

    def w1(j, paced):
        def act(r0, i, val):
            c0 = LANE + half(j, i % 2).start
            h_ref[quad(r0, GRP, i), c0:c0 + TH] = _gelu(val)
        _matmul(a_1, b_d, j, GRP, act, paced=paced)

    def shift(j):
        def shifted(rows, n):
            by = SHIFTS[rows.start // GRP]
            lo = half(j, n).start + (0 if by > 0 else LANE)
            off = LANE - by if by > 0 else -by
            return h_ref[rows, lo:lo + TH + LANE][:, off:off + TH]
        for r0 in range(0, D2, 16):
            _put_rhs(b_d, j, r0, 0, *[shifted(quad(r0, 16, i), i % 2) for i in range(4)])

    def w2(j, paced):
        def add(r0, i, val):
            rows, cs = quad(r0, D2, i), half(j, i % 2)
            x1 = (x_ref[rows, cs] - stat_ref[0:1, cs]) * stat_ref[1:2, cs] + val
            y_ref[rows, cs] = x1
            note(j, i % 2, x1)
        _matmul(a_2, b_d, j, D2, add, paced=paced)

    def w3(j, paced):
        def staged(r0):
            return g_ref[(4 * j + (r0 + LANE) // HID) % 3]

        def act(r0, i, val):
            staged(r0)[i, 0:val.shape[0], :] = _gelu(val)

        def operands(r0, rows):
            def step(rr, t, i, gate):
                def quadrant(q):
                    return [staged(r0)[q, r:r + 32, c0:c0 + LANE] for r in range(rr, rows, LANE) for c0 in (t, t + TH // 2)]
                u, v, sign = ((0, None, 0), (2, 0, -1), (3, None, 0), (0, 3, 1), (2, 3, 1), (1, 3, -1), (0, 1, 1))[i]
                x = [part if n in (1, 2) else after(part, gate) for n, part in enumerate(quadrant(u))]
                if v is not None:
                    x = [a + b if sign > 0 else a - b for a, b in zip(x, quadrant(v))]
                if rows == LANE:
                    ops, dst = (x[0], None, None, x[0], None, x[1], x[0] + x[1]), FB
                else:
                    ops, dst = _rhs(*x), (r0 - LANE) // 2
                for k, op in enumerate(ops):
                    if op is not None:
                        _put(b_f[j], (i, k), dst + rr, t, op)
            return [lambda gate, rr=rr, t=t, i=i: step(rr, t, i, gate)
                    for rr in range(0, LANE, 32) for t in range(0, TH // 2, LANE) for i in range(7)]
        return _matmul(a_3, b_d, j, HID, act, later=operands, paced=paced)

    def w4(j, last, paced):
        def add(r0, i, val):
            at = quad(r0, D2, i), half(j, i % 2)
            x = (x_ref[at] + y_ref[at]) + val
            if last:
                io_buf[at] = x.astype(bf16)
                out_copy(j, i).start()
            else:
                x_ref[at] = x
                note(j, i % 2, x)
        _matmul(a_4, b_f[j], j, D2, add, paced=paced)

    def transposed_halves(w_ref, cs, gate):
        return [after(w_ref[r:r + D2, cs].astype(f32), gate).T for r in (0, D2)]

    def prep_qkv(i, gate):
        qkv_cp[i].wait()
        c0 = (1, 0, 2)[i] * D
        lo = c0 // LANE * LANE
        wl, wr = transposed_halves(wqkv_in, slice(lo, min(pl.cdiv(c0 + D, LANE) * LANE, 3 * D)), gate)
        r = c0 - lo
        _put_lhs(a_qkv, i * D2, wl[r:r + D2], wr[r:r + D2], wl[r + D2:r + D], wr[r + D2:r + D])

    def prep_o(gate):
        halves = []
        for r in (0, D2):
            w = after(wo_in[r:r + D2, :].astype(f32), gate)
            wins = [jnp.where(_own_rows(h, D), w[_win_start(h):_win_start(h) + WIN], 0.0) for h in range(H // 2)]
            halves.append(jnp.concatenate(wins, axis=0).T)
        wl, wr = halves
        _put_lhs(a_o, 0, wl[0:D2], wr[0:D2], wl[D2:D], wr[D2:D])

    def prep_square(w_ref, a_ref, gate):
        wl, wr = transposed_halves(w_ref, slice(None), gate)
        _put_lhs(a_ref, 0, wl[0:D2], wr[0:D2], wl[D2:D], wr[D2:D])

    def prep_3(t, gate):
        blocks = [v for c0 in (t * LANE, F2 + t * LANE) for v in transposed_halves(w3_in, slice(c0, c0 + LANE), gate)]
        _put_lhs(a_3, (1, 3, 5, 0, 2, 4, 6)[t] * LANE, *blocks)

    def prep_4(r0, c0, i, gate):
        def part(q, c):
            def blk(n):
                return w4_in[quad(q * GRP + r0, 16, n), n % 2 * F2 + c:n % 2 * F2 + c + LANE].astype(f32)
            u, v, sign = ((2, 3, 1), (3, None, 0), (0, 1, 1), (0, 3, 1), (1, 3, -1), (0, None, 0), (2, 0, -1))[i]
            y = after(blk(u), gate)
            return y if v is None else y + blk(v) if sign > 0 else y - blk(v)
        y11, y21 = part(0, c0), part(1, c0)
        if c0 < FB:
            ops = _lhs(y11, part(0, FA + c0), y21, part(1, FA + c0))
        else:
            ops = (y21, None, None, y11, None, y11, y21 - y11)
        for k, op in enumerate(ops):
            if op is not None:
                _put(a_4, (i, k), r0, c0, op)

    def prep_rest():
        gap = [lambda gate: None] * 15
        steps = ([prep_o] + gap * 2 + [lambda gate: prep_square(w1_in, a_1, gate)] + gap * 2
                 + [lambda gate: prep_square(w2_in, a_2, gate)] + gap * 2)
        for t in range(F2 // LANE):
            steps += [lambda gate, t=t: prep_3(t, gate)] + gap
        return steps + [lambda gate, r0=r0, c0=c0, i=i: prep_4(r0, c0, i, gate)
                        for r0 in range(0, GRP, 16) for c0 in range(0, FA, LANE) for i in range(7)]

    def rest_of_round(top, last, side):
        n = 2 * NW - 2
        units = [unit(H // 2 - 1, u, top, 2 * NW - 1 - u, side[u * len(side) // n:(u + 1) * len(side) // n])
                 for u in range(2 * NW)]
        for u in range(2 * NW - 1):
            for step in units[u]:
                step()
            if u == NW:
                for j in range(2):
                    for i in range(H // 2 - 1):
                        o_operands(j, i)
            if u == NW + 1:
                o_operands(0, H // 2 - 1)
        wo(0, [(units[-1], (0.0, 0.7))])
        o_operands(1, H // 2 - 1)
        span = (0.05, 0.7)
        wo(1, [(layernorm(0, x_ref, twice=True), span)])
        w1(0, [(layernorm(1, x_ref, twice=True), span)])
        w1(1, [])
        shift(0)
        shift(1)
        w2(0, [])
        w2(1, [(layernorm(0, y_ref), span)])
        fence()
        todo = w3(0, [(layernorm(1, y_ref), (0.02, 0.28))])
        todo = w3(1, [(todo, (0.0, 0.45))])
        w4(0, last, [(todo, (0.0, 0.45))])
        w4(1, last, [] if last else [(layernorm(0, x_ref), (0.05, 0.8))])

    qkv_cp[0].start()
    x_cp[0].start()
    fence()
    h_ref[:, 0:LANE] = jnp.zeros((D, LANE), f32)
    h_ref[:, LANE + S:] = jnp.zeros((D, LANE), f32)
    prep_qkv(0, None)
    x_cp[0].wait()
    for cp in (qkv_cp[1], qkv_cp[2], x_cp[1]):
        cp.start()
    widen_input(0)
    for step in layernorm(0, x_ref):
        step(None)

    def arrivals(gate):
        x_cp[1].wait()
        prep_qkv(2, gate)
        widen_input(1)
    qkv(0, [([lambda gate: prep_qkv(1, gate), arrivals], (0.15, 0.85)), (layernorm(1, x_ref), (0.6, 0.92))])
    qkv(1, [])
    for cp in w_cp:
        cp.start()
    top = attention_loop()
    for cp in w_cp:
        cp.wait()
    rest_of_round(top, False, prep_rest())

    fence()
    qkv(0, [(layernorm(1, x_ref), (0.1, 0.8))])
    qkv(1, [])
    rest_of_round(attention_loop(), True, [])
    for j in range(2):
        for i in range(4):
            out_copy(j, i).wait()


@jax.jit
def pallas_interleave_layers__mha_block__mixer_s_mlp__prompt_kernel(
    A_x: jax.Array,
    A_wqkv: jax.Array,
    A_wo: jax.Array,
    B_x: jax.Array,
    B_w1: jax.Array,
    B_w2: jax.Array,
    B_w3: jax.Array,
    B_w4: jax.Array,
):
    del B_x
    in_hbm = pl.BlockSpec(memory_space=pl.ANY)
    out = pl.pallas_call(
        _kernel,
        out_shape=jax.ShapeDtypeStruct((D, S), bf16),
        in_specs=[in_hbm] * 7,
        out_specs=in_hbm,
        scratch_shapes=[
            pltpu.VMEM((D, S), bf16),
            pltpu.VMEM((D, 3 * D), bf16),
            pltpu.VMEM((D, D), bf16),
            pltpu.VMEM((D, D), bf16),
            pltpu.VMEM((D, D), bf16),
            pltpu.VMEM((D, F), bf16),
            pltpu.VMEM((D, F), bf16),
            pltpu.VMEM((7, 2, 3 * D2, LANE), bf16),
            pltpu.VMEM((7, 2, D2, LANE), bf16),
            pltpu.VMEM((7, 2, D2, LANE), bf16),
            pltpu.VMEM((7, 2, D2, LANE), bf16),
            pltpu.VMEM((7, 2, F2, LANE), bf16),
            pltpu.VMEM((7, 7, FA // LANE, GRP, LANE), bf16),
            pltpu.VMEM((2, 7, TH // LANE, D2, LANE), bf16),
            pltpu.VMEM((2, 7, TH // LANE, H * WIN // 2, LANE), bf16),
            pltpu.VMEM((7, 7, TH // 2 // LANE, FA, LANE), bf16),
            pltpu.VMEM((7, 7, TH // 2 // LANE, FA, LANE), bf16),
            pltpu.VMEM((4, HID, TH), f32),
            pltpu.VMEM((4, HID, TH), f32),
            pltpu.VMEM((4, HID, TH), f32),
            pltpu.VMEM((2, 8, LANE), f32),
            pltpu.VMEM((8, S), f32),
            pltpu.VMEM((D, S), f32),
            pltpu.VMEM((D, S), f32),
            pltpu.VMEM((H, S // LANE, WIN, LANE), bf16),
            pltpu.VMEM((H, 1, S, LANE), bf16),
            pltpu.VMEM((H, S // LANE, WIN, LANE), bf16),
            pltpu.VMEM((H * NW, WIN, W), f32),
            pltpu.VMEM((S, W), f32),
            pltpu.VMEM((S, W), f32),
            pltpu.VMEM((D, S + 2 * LANE), f32),
            pltpu.SemaphoreType.DMA((10,)),
            pltpu.SemaphoreType.DMA((8,)),
        ],
        compiler_params=pltpu.CompilerParams(vmem_limit_bytes=124 * 2 ** 20),
        name='fused',
    )(A_x[0].T, A_wqkv, A_wo, B_w1, B_w2, B_w3, B_w4.T)
    return out.T[None]
```
